```python
import os as _os
_os.environ.setdefault("JAX_PLATFORMS", "cpu")
import jax
import jax.numpy as jnp

def _softmax(x, axis=-1):
    return jax.nn.softmax(x, axis=axis)
def _gelu(x):
    return jax.nn.gelu(x, approximate=True)
def _silu(x):
    return jax.nn.silu(x)
def _sigmoid(x):
    return jax.nn.sigmoid(x)
def _layernorm(x, axis=-1, eps=1e-5):
    m = jnp.mean(x, axis=axis, keepdims=True)
    v = jnp.var(x, axis=axis, keepdims=True)
    return (x - m) / jnp.sqrt(v + eps)
def _scatter_add(tgt, idx, src, axis=0):
    return tgt.at[idx].add(src)
def _segment_sum(src, seg, n):
    return jax.ops.segment_sum(src, seg, n)
class _Rng:
    def __init__(self, key):
        self._k = key
    def _next(self):
        self._k, sub = jax.random.split(self._k)
        return sub
    def normal(self, shape):
        return jax.random.normal(self._next(), shape, dtype=jnp.bfloat16)
    def randint(self, lo, hi, shape):
        return jax.random.randint(self._next(), shape, lo, hi, dtype=jnp.int32)
    def uniform(self, shape, lo=0.0, hi=1.0):
        return jax.random.uniform(self._next(), shape, jnp.bfloat16, lo, hi)
    def permutation(self, n):
        return jax.random.permutation(self._next(), n)


kernel_name = 'sequential_preLN__linear_attn_block__glu_gated_reglu__prompt'

def setup_inputs():
    _rng = _Rng(jax.random.key(int.from_bytes(__import__("os").urandom(4), "little")))
    _w = (lambda a: (lambda t: t.astype(jnp.bfloat16) if jnp.issubdtype(t.dtype, jnp.floating) else t)(jnp.asarray(a)))
    def _A_setup():
        B, S, D = 1, 2048, 640
        return {
            "x": _w((lambda *s: _rng.normal(s) * 0.05)(B, S, D)),
            "wqkv": _w((lambda *s: _rng.normal(s) * 0.05)(D, 3 * D)),
            "wo": _w((lambda *s: _rng.normal(s) * 0.05)(D, D)),
        }
    _A_in = _A_setup()

    def _B_setup():
        B, S, D, F = 1, 2048, 640, 1536
        return {
            "x": _w((lambda *s: _rng.normal(s) * 0.05)(B, S, D)),
            "W_gate": _w((lambda *s: _rng.normal(s) * 0.05)(D, F) * (2.0 / D) ** 0.5),
            "W_up": _w((lambda *s: _rng.normal(s) * 0.05)(D, F) * (2.0 / D) ** 0.5),
            "W_down": _w((lambda *s: _rng.normal(s) * 0.05)(F, D) * (1.0 / F) ** 0.5),
        }
    _B_in = _B_setup()

    return {
        "A_x": _A_in["x"],
        "A_wqkv": _A_in["wqkv"],
        "A_wo": _A_in["wo"],
        "B_x": _B_in["x"],
        "B_W_gate": _B_in["W_gate"],
        "B_W_up": _B_in["W_up"],
        "B_W_down": _B_in["W_down"],
    }

def reference(A_x, A_wqkv, A_wo, B_x, B_W_gate, B_W_up, B_W_down):
    def _A_ref(x, wqkv, wo):
        B, S, D = x.shape
        H = 32; Dh = D // H
        qkv = (lambda x, *d: x.transpose(*d))((x @ wqkv).reshape(B, S, 3, H, Dh), 2, 0, 3, 1, 4)
        q, k, v = qkv[0], qkv[1], qkv[2]
        phi = lambda t: jnp.where(t > 0, t + 1, jnp.exp(t)) + 1e-6
        pq, pk = phi(q), phi(k)
        kv = jnp.einsum("bhsd,bhse->bhde", pk, v)
        z = jnp.einsum("bhsd->bhd", pk)
        num = jnp.einsum("bhqd,bhde->bhqe", pq, kv)
        den = jnp.einsum("bhqd,bhd->bhq", pq, z)[..., None] + 1e-6
        o = num / den
        return (lambda x, *d: x.transpose(*d))(o, 0, 2, 1, 3).reshape(B, S, D) @ wo

    def _B_ref(x, W_gate, W_up, W_down):
        gate = jnp.einsum("bsd,df->bsf", x, W_gate)
        up = jnp.einsum("bsd,df->bsf", x, W_up)
        gate = gate * (lambda x, dt: x.astype(dt))(gate > 0, gate.dtype)
        h = gate * up
        return jnp.einsum("bsf,fd->bsd", h, W_down)

    x = A_x
    h = x + _A_ref(_layernorm(x, axis=-1), A_wqkv, A_wo)
    h2 = h + _B_ref(_layernorm(h, axis=-1), B_W_gate, B_W_up, B_W_down)
    return h2
```

```python
import functools
import jax
import jax.numpy as jnp
from jax import lax
import jax.experimental.pallas as pl
import jax.experimental.pallas.tpu as pltpu

S, D, F = 2048, 640, 1536
H, DH = 32, 20
TM = 256
NB = S // TM
FC = 512
KC = D // 128
LN_EPS = 1e-5
EPS = 1e-6
_NT = (((1,), (1,)), ((), ()))


def _row_windows():
    wins = []
    for j in range(D // 128):
        h0 = (128 * j) // DH
        h1 = (128 * j + 127) // DH
        r0 = (h0 * DH) // 16 * 16
        r1 = -(-((h1 + 1) * DH) // 16) * 16
        wins.append((r0, r1))
    return wins

WINS = _row_windows()


def _ln(x):
    m = jnp.mean(x, axis=-1, keepdims=True)
    xc = x - m
    v = jnp.mean(xc * xc, axis=-1, keepdims=True)
    return xc * lax.rsqrt(v + LN_EPS)


def _phi(t):
    return jnp.where(t > 0, t + 1.0, jnp.exp(t)) + EPS


def _head(i):
    return (i * 3277) >> 16


def _permute_rows(dst, src, cols, dtype):
    for m in range(DH):
        dst[32 * m:32 * (m + 1), cols] = src[pl.ds(m, H, stride=DH), :].astype(dtype)


def _normalize(pq, zrow):
    t = pq * zrow
    s = t[:, 0:128]
    for j in range(1, D // 128):
        s = s + t[:, 128 * j:128 * (j + 1)]
    s = s + pltpu.roll(s, 32, 1)
    s = s + pltpu.roll(s, 64, 1)
    rec = 1.0 / (s + EPS)
    parts = [(pq[:, 128 * j:128 * (j + 1)] * rec).astype(jnp.bfloat16) for j in range(D // 128)]
    return jnp.concatenate(parts, axis=1)


def _kernel(x_hbm, wqkv_hbm, wo_hbm, wg_hbm, wu_hbm, wd_hbm, out_hbm,
            x_v, wqkv_v, wo_v, wg_v, wu_v, wd_v, out_v,
            wkt_v, wqt_v, tq_v, xn_all, h_buf, hn_buf, pkt_buf, v_buf,
            q_acc, v_acc, kt_acc,
            kv_v, zacc_v, zp_v, zrow_v, mf_v, m_v,
            xsem, csem, wsem, osem):
    f32, bf16 = jnp.float32, jnp.bfloat16

    def x_copy(i):
        return pltpu.make_async_copy(x_hbm.at[0, pl.ds(i * TM, TM), :], x_v.at[pl.ds(i * TM, TM), :], xsem.at[i])

    def o_copy(i):
        return pltpu.make_async_copy(out_v.at[pl.ds(i * TM, TM), :], out_hbm.at[0, pl.ds(i * TM, TM), :], osem.at[i])

    def c_copy(c):
        return pltpu.make_async_copy(wqkv_hbm.at[pl.ds(128 * c, 128), :], wqkv_v.at[pl.ds(128 * c, 128), :], csem.at[c])

    c_wo = pltpu.make_async_copy(wo_hbm, wo_v, wsem.at[0])
    c_wg = pltpu.make_async_copy(wg_hbm, wg_v, wsem.at[1])
    c_wu = pltpu.make_async_copy(wu_hbm, wu_v, wsem.at[2])
    c_wd = pltpu.make_async_copy(wd_hbm, wd_v, wsem.at[3])

    x_copy(0).start()
    c_copy(0).start()
    c_copy(1).start()

    kv_v[...] = jnp.zeros_like(kv_v)

    def prep1(i):
        r = pl.multiple_of(i * TM, TM)
        xn_all[pl.ds(r, TM), :] = _ln(x_v[pl.ds(r, TM), :].astype(f32)).astype(bf16)

    def kvacc(pkt, v):
        for j, (r0, r1) in enumerate(WINS):
            kv_v[r0:r1, 128 * j:128 * (j + 1)] += jnp.dot(
                pkt[r0:r1, :], v[:, 128 * j:128 * (j + 1)], preferred_element_type=f32)

    def zfold(pkt):
        zs = pkt[:, 0:128]
        for c in range(1, TM // 128):
            zs = zs + pkt[:, 128 * c:128 * (c + 1)]
        return zs

    def kqpart(c):
        kp = slice(128 * c, 128 * (c + 1))
        xc = xn_all[0:TM, kp]
        for hh in range(2):
            rs = slice(hh * (D // 2), (hh + 1) * (D // 2))
            ktp = lax.dot_general(wkt_v[rs, kp], xc, _NT, preferred_element_type=f32)
            if c == 0:
                kt_acc[rs, :] = ktp
            else:
                kt_acc[rs, :] += ktp
        qp = lax.dot_general(xc, wqt_v[:, kp], _NT, preferred_element_type=f32)
        if c == 0:
            q_acc[...] = qp
        else:
            q_acc[...] += qp

    x_copy(0).wait()
    prep1(0)
    for c in range(KC):
        c_copy(c).wait()
        if c + 2 < KC:
            c_copy(c + 2).start()
        elif c + 2 == KC:
            x_copy(1).start()
        else:
            for i in range(2, NB):
                x_copy(i).start()
            c_wo.start()
            c_wg.start()
            c_wu.start()
            c_wd.start()
        ks = slice(128 * c, 128 * (c + 1))
        if c == KC - 1:
            x_copy(1).wait()
            prep1(1)
        if c > 0:
            kqpart(c - 1)
        wkt_v[:, ks] = wqkv_v[ks, D:2 * D].astype(f32).T.astype(bf16)
        tq_v[...] = wqkv_v[ks, 0:D].astype(f32).T
        _permute_rows(wqt_v, tq_v, ks, bf16)
        vp = jnp.dot(xn_all[0:TM, ks], wqkv_v[ks, 2 * D:3 * D], preferred_element_type=f32)
        if c == 0:
            v_acc[...] = vp
        else:
            v_acc[...] += vp
    kqpart(KC - 1)
    pkt0 = _phi(kt_acc[...])
    zacc_v[...] = zfold(pkt0)
    pkt_buf[0] = pkt0.astype(bf16)
    v_buf[0] = v_acc[...].astype(bf16)

    def phase1(i, carry):
        s = i % 2

        @pl.when(i + 1 < NB)
        def _():
            x_copy(i + 1).wait()
        r = pl.multiple_of(i * TM, TM)
        xn = xn_all[pl.ds(r, TM), :]
        pkt_prev = pkt_buf[1 - s]
        v_prev = v_buf[1 - s]
        prep1(jnp.minimum(i + 1, NB - 1))
        pkt = _phi(lax.dot_general(wkt_v[...], xn, _NT, preferred_element_type=f32))
        zacc_v[...] += zfold(pkt)
        pkt_buf[s] = pkt.astype(bf16)
        kvacc(pkt_prev, v_prev)
        v_buf[s] = jnp.dot(xn, wqkv_v[:, 2 * D:3 * D], preferred_element_type=f32).astype(bf16)
        return carry

    lax.fori_loop(1, NB, phase1, 0)

    c_wo.wait()
    sl = (NB - 1) % 2
    kvacc(pkt_buf[sl], v_buf[sl])
    _permute_rows(zp_v, zacc_v, slice(None), f32)
    zrow = jnp.sum(zp_v[...].T, axis=0, keepdims=True)
    zrow_v[...] = jnp.broadcast_to(zrow, zrow_v.shape)
    pqn0 = _normalize(_phi(q_acc[...]), zrow)
    parts = []
    for j, (r0, r1) in enumerate(WINS):
        rows = lax.broadcasted_iota(jnp.int32, (r1 - r0, 128), 0) + r0
        cols = lax.broadcasted_iota(jnp.int32, (r1 - r0, 128), 1) + 128 * j
        kvm = jnp.where(_head(rows) == _head(cols), kv_v[r0:r1, 128 * j:128 * (j + 1)], 0.0).astype(bf16)
        parts.append(jnp.dot(kvm, wo_v[128 * j:128 * (j + 1), :], preferred_element_type=f32))
    for j, (r0, r1) in enumerate(WINS):
        lo = WINS[j - 1][1] if j > 0 else r0
        hi = WINS[j + 1][0] if j + 1 < len(WINS) else r1
        for n in range(D // 128):
            ns = slice(128 * n, 128 * (n + 1))
            mf_v[n, lo:hi, :] = parts[j][lo - r0:hi - r0, ns]
            if j + 1 < len(WINS):
                n0 = WINS[j + 1][0]
                mf_v[n, hi:r1, :] = parts[j][hi - r0:r1 - r0, ns] + parts[j + 1][0:r1 - n0, ns]
    for n in range(D // 128):
        _permute_rows(m_v, mf_v.at[n], slice(128 * n, 128 * (n + 1)), bf16)
    h0 = x_v[0:TM, :].astype(f32) + jnp.dot(pqn0, m_v[...], preferred_element_type=f32)
    h_buf[0] = h0
    hn_buf[0] = _ln(h0).astype(bf16)
    c_wg.wait()
    c_wu.wait()
    c_wd.wait()

    def gu(hn, c):
        g = jnp.dot(hn, wg_v[:, c * FC:(c + 1) * FC], preferred_element_type=f32)
        u = jnp.dot(hn, wu_v[:, c * FC:(c + 1) * FC], preferred_element_type=f32)
        return (jnp.maximum(g, 0.0) * u).astype(bf16)

    def down(a, c):
        return jnp.dot(a, wd_v[c * FC:(c + 1) * FC, :], preferred_element_type=f32)

    def phase2(i, carry):
        s = i % 2
        r = pl.multiple_of(i * TM, TM)
        rn = pl.multiple_of((i + 1) * TM, TM)
        hn = hn_buf[s]
        hcur = h_buf[s]
        xn = xn_all[pl.ds(rn, TM), :]
        pq = _phi(lax.dot_general(xn, wqt_v[...], _NT, preferred_element_type=f32))
        pqn = _normalize(pq, zrow_v[0:1, :])
        a0 = gu(hn, 0)
        acc = hcur + down(a0, 0)
        attn = jnp.dot(pqn, m_v[...], preferred_element_type=f32)
        h = x_v[pl.ds(rn, TM), :].astype(f32) + attn
        h_buf[1 - s] = h
        hn_buf[1 - s] = _ln(h).astype(bf16)
        a1 = gu(hn, 1)
        acc = acc + down(a1, 1)
        a2 = gu(hn, 2)
        acc = acc + down(a2, 2)
        out_v[pl.ds(r, TM), :] = acc.astype(bf16)
        o_copy(i).start()
        return carry

    lax.fori_loop(0, NB - 1, phase2, 0)
    hn = hn_buf[sl]
    acc = h_buf[sl]
    for c in range(F // FC):
        acc = acc + down(gu(hn, c), c)
    out_v[pl.ds((NB - 1) * TM, TM), :] = acc.astype(bf16)
    o_copy(NB - 1).start()
    for i in range(NB):
        o_copy(i).wait()


@jax.jit
def pallas_sequential_preLN__linear_attn_block__glu_gated_reglu__prompt_kernel(
    A_x, A_wqkv, A_wo, B_x, B_W_gate, B_W_up, B_W_down):
    bf16, f32 = jnp.bfloat16, jnp.float32
    any_spec = pl.BlockSpec(memory_space=pl.ANY)
    return pl.pallas_call(
        _kernel,
        out_shape=jax.ShapeDtypeStruct((1, S, D), bf16),
        in_specs=[any_spec] * 6,
        out_specs=any_spec,
        scratch_shapes=[
            pltpu.VMEM((S, D), bf16),
            pltpu.VMEM((D, 3 * D), bf16),
            pltpu.VMEM((D, D), bf16),
            pltpu.VMEM((D, F), bf16),
            pltpu.VMEM((D, F), bf16),
            pltpu.VMEM((F, D), bf16),
            pltpu.VMEM((S, D), bf16),
            pltpu.VMEM((D, D), bf16),
            pltpu.VMEM((D, D), bf16),
            pltpu.VMEM((D, 128), f32),
            pltpu.VMEM((S, D), bf16),
            pltpu.VMEM((2, TM, D), f32),
            pltpu.VMEM((2, TM, D), bf16),
            pltpu.VMEM((2, D, TM), bf16),
            pltpu.VMEM((2, TM, D), bf16),
            pltpu.VMEM((TM, D), f32),
            pltpu.VMEM((TM, D), f32),
            pltpu.VMEM((D, TM), f32),
            pltpu.VMEM((D, D), f32),
            pltpu.VMEM((D, 128), f32),
            pltpu.VMEM((D, 128), f32),
            pltpu.VMEM((8, D), f32),
            pltpu.VMEM((D // 128, D, 128), f32),
            pltpu.VMEM((D, D), bf16),
            pltpu.SemaphoreType.DMA((NB,)),
            pltpu.SemaphoreType.DMA((KC,)),
            pltpu.SemaphoreType.DMA((4,)),
            pltpu.SemaphoreType.DMA((NB,)),
        ],
        compiler_params=pltpu.CompilerParams(vmem_limit_bytes=64 * 1024 * 1024),
    )(A_x, A_wqkv, A_wo, B_W_gate, B_W_up, B_W_down)
```

```python
import jax
import jax.numpy as jnp
from jax import lax
import jax.experimental.pallas as pl
import jax.experimental.pallas.tpu as pltpu

S, D, F = 2048, 640, 1536
H, DH = 32, 20
TM = 256
NB = S // TM
FC = 512
KC = D // 128
RC = 32
TAIL = ((0, 112), (112, 192), (192, 240), (240, 256))
LN_EPS = 1e-5
EPS = 1e-6
_NT = (((1,), (1,)), ((), ()))


def _row_windows():
    wins = []
    for j in range(D // 128):
        h0 = (128 * j) // DH
        h1 = (128 * j + 127) // DH
        r0 = (h0 * DH) // 16 * 16
        r1 = -(-((h1 + 1) * DH) // 16) * 16
        wins.append((r0, r1))
    return wins


WINS = _row_windows()


def _ln(x):
    m = jnp.mean(x, axis=-1, keepdims=True)
    xc = x - m
    v = jnp.mean(xc * xc, axis=-1, keepdims=True)
    return xc * lax.rsqrt(v + LN_EPS)


def _phi(t):
    return jnp.where(t > 0, t + 1.0, jnp.exp(t)) + EPS


def _head(i):
    return (i * 3277) >> 16


def _permute_rows(dst, src, cols, dtype):
    for m in range(DH):
        dst[32 * m:32 * (m + 1), cols] = src[pl.ds(m, H, stride=DH), :].astype(dtype)


def _normalize(pq, zrow):
    t = pq * zrow
    s = t[:, 0:128]
    for j in range(1, D // 128):
        s = s + t[:, 128 * j:128 * (j + 1)]
    s = s + pltpu.roll(s, 32, 1)
    s = s + pltpu.roll(s, 64, 1)
    rec = 1.0 / (s + EPS)
    parts = [(pq[:, 128 * j:128 * (j + 1)] * rec).astype(jnp.bfloat16) for j in range(D // 128)]
    return jnp.concatenate(parts, axis=1)


def _kernel(x_hbm, wqkv_hbm, wo_hbm, wg_hbm, wu_hbm, wd_hbm, out_hbm,
            x_v, wq_v, wkv_v, wo_v, wg_v, wu_v, wd_v, out_v,
            wkt_v, wqt_v, tq_v, xn_all, h_buf, hn_buf, xn_0, xn_1, pkt_0, pkt_1, v_0, v_1,
            v_acc, kt_acc,
            kv_v, zacc_v, zp_v, zrow_v, mf_v, m_v,
            xsem, csem, wsem, osem):
    f32, bf16 = jnp.float32, jnp.bfloat16

    def x_copy(i):
        return pltpu.make_async_copy(x_hbm.at[0, pl.ds(i * TM, TM), :], x_v.at[pl.ds(i * TM, TM), :], xsem.at[0])

    def x2_copy(j):
        r = (2 * j + 2) * TM
        return pltpu.make_async_copy(x_hbm.at[0, pl.ds(r, 2 * TM), :], x_v.at[pl.ds(r, 2 * TM), :], xsem.at[1 + j])

    def o_copy(r, n):
        return pltpu.make_async_copy(out_v.at[pl.ds(r, n), :], out_hbm.at[0, pl.ds(r, n), :], osem.at[0])

    def c_copy(c):
        return pltpu.make_async_copy(wqkv_hbm.at[pl.ds(128 * c, 128), pl.ds(D, 2 * D)],
                                     wkv_v.at[pl.ds(128 * c, 128), :], csem.at[c % 2])

    c_wq = pltpu.make_async_copy(wqkv_hbm.at[:, pl.ds(0, D)], wq_v, wsem.at[0])
    c_wo = pltpu.make_async_copy(wo_hbm, wo_v, wsem.at[0])
    c_wg = pltpu.make_async_copy(wg_hbm, wg_v, wsem.at[1])
    c_wu = pltpu.make_async_copy(wu_hbm, wu_v, wsem.at[1])
    c_wd = pltpu.make_async_copy(wd_hbm, wd_v, wsem.at[1])

    x_copy(0).start()
    c_copy(0).start()

    kv_v[...] = jnp.zeros_like(kv_v)

    def prep1(i, dst, chain=False):
        tok = None
        for k in range(TM // RC):
            r = pl.multiple_of(i * TM + k * RC, RC)
            x = x_v[pl.ds(r, RC), :].astype(f32)
            if tok is not None:
                x = jnp.concatenate([x[:, :D - 128], x[:, D - 128:] + tok], axis=1)
            xn = _ln(x)
            if chain:
                tok = xn[:, D - 128:] * 0.0
            xn = xn.astype(bf16)
            dst[k * RC:(k + 1) * RC, :] = xn
            xn_all[pl.ds(r, RC), :] = xn

    def resid_ln(i, slot, attn, row0=0):
        for k in range(attn.shape[0] // RC):
            r = pl.multiple_of(i * TM + row0 + k * RC, RC)
            h = x_v[pl.ds(r, RC), :].astype(f32) + attn[k * RC:(k + 1) * RC, :]
            h_buf[slot, row0 + k * RC:row0 + (k + 1) * RC, :] = h
            hn_buf[slot, row0 + k * RC:row0 + (k + 1) * RC, :] = _ln(h).astype(bf16)

    def kvacc(pkt, v):
        for j, (r0, r1) in enumerate(WINS):
            kv_v[r0:r1, 128 * j:128 * (j + 1)] += jnp.dot(
                pkt[r0:r1, :], v[:, 128 * j:128 * (j + 1)], preferred_element_type=f32)

    def zfold(pkt):
        zs = pkt[:, 0:128]
        for c in range(1, TM // 128):
            zs = zs + pkt[:, 128 * c:128 * (c + 1)]
        return zs

    def acc_store(ref, idx, val, first):
        if first:
            ref[idx] = val
        else:
            ref[idx] += val

    def kpart(c):
        kp = slice(128 * c, 128 * (c + 1))
        xc = xn_0[:, kp]
        for hh in range(2):
            rs = slice(hh * (D // 2), (hh + 1) * (D // 2))
            acc_store(kt_acc, (rs, slice(None)),
                      lax.dot_general(wkt_v[rs, kp], xc, _NT, preferred_element_type=f32), c == 0)

    def vpart(c):
        kp = slice(128 * c, 128 * (c + 1))
        xc = xn_0[:, kp]
        acc_store(v_acc, (slice(None), slice(0, D - 128)),
                  jnp.dot(xc, wkv_v[kp, D:2 * D - 128], preferred_element_type=f32), c == 0)
        for hh in range(4):
            rs = slice(hh * (TM // 4), (hh + 1) * (TM // 4))
            acc_store(v_acc, (rs, slice(D - 128, D)),
                      jnp.dot(xc[rs, :], wkv_v[kp, 2 * D - 128:2 * D], preferred_element_type=f32), c == 0)

    def kproj(xn, pkt_dst):
        pkt = _phi(lax.dot_general(wkt_v[...], xn, _NT, preferred_element_type=f32))
        zacc_v[...] += zfold(pkt)
        pkt_dst[...] = pkt.astype(bf16)

    def vproj(xn, v_dst):
        v_dst[...] = jnp.dot(xn, wkv_v[:, D:2 * D], preferred_element_type=f32).astype(bf16)

    def qproj(xn):
        return _phi(lax.dot_general(xn, wqt_v[...], _NT, preferred_element_type=f32))

    x_copy(0).wait()
    c_copy(1).start()
    prep1(0, xn_0)
    for c in range(KC):
        c_copy(c).wait()
        if c + 2 < KC:
            c_copy(c + 2).start()
        elif c + 2 == KC:
            x_copy(1).start()
        else:
            x2_copy(0).start()
        ks = slice(128 * c, 128 * (c + 1))
        if c == KC - 1:
            x_copy(1).wait()
            x2_copy(1).start()
            x2_copy(2).start()
            prep1(1, xn_1)
        vpart(c)
        if c > 0:
            kpart(c - 1)
        wkt_v[:, ks] = wkv_v[ks, 0:D].astype(f32).T.astype(bf16)
    kpart(KC - 1)
    pkt0 = _phi(kt_acc[...])
    zacc_v[...] = zfold(pkt0)
    pkt_0[...] = pkt0.astype(bf16)
    v_0[...] = v_acc[...].astype(bf16)

    c_wq.start()
    c_wo.start()
    c_wg.start()
    c_wu.start()
    c_wd.start()

    def step1(xn_c, pkt_c, v_c, pkt_p, v_p):
        xn = xn_c[...]
        kvacc(pkt_p, v_p)
        kproj(xn, pkt_c)
        vproj(xn, v_c)

    def phase1(j, carry):
        x2_copy(j).wait()
        prep1(2 * j + 2, xn_0, chain=True)
        step1(xn_1, pkt_1, v_1, pkt_0, v_0)
        prep1(2 * j + 3, xn_1, chain=True)
        step1(xn_0, pkt_0, v_0, pkt_1, v_1)
        return carry

    lax.fori_loop(0, NB // 2 - 1, phase1, 0)

    c_wq.wait()
    c_wo.wait()
    for c in range(KC):
        ks = slice(128 * c, 128 * (c + 1))
        tq_v[c] = wq_v[ks, :].astype(f32).T
        _permute_rows(wqt_v, tq_v.at[c], ks, bf16)
    xn = xn_1[...]
    kvacc(pkt_0, v_0)
    kproj(xn, pkt_1)
    pq0 = [qproj(xn_all[0:TM // 2, :])]
    vproj(xn, v_1)
    kvacc(pkt_1, v_1)

    _permute_rows(zp_v, zacc_v, slice(None), f32)
    zrow = jnp.sum(zp_v[...].T, axis=0, keepdims=True)
    zrow_v[...] = jnp.broadcast_to(zrow, zrow_v.shape)
    parts = []
    for j, (r0, r1) in enumerate(WINS):
        rows = lax.broadcasted_iota(jnp.int32, (r1 - r0, 128), 0) + r0
        cols = lax.broadcasted_iota(jnp.int32, (r1 - r0, 128), 1) + 128 * j
        kvm = jnp.where(_head(rows) == _head(cols), kv_v[r0:r1, 128 * j:128 * (j + 1)], 0.0).astype(bf16)
        parts.append(jnp.dot(kvm, wo_v[128 * j:128 * (j + 1), :], preferred_element_type=f32))
    for j, (r0, r1) in enumerate(WINS):
        lo = WINS[j - 1][1] if j > 0 else r0
        hi = WINS[j + 1][0] if j + 1 < len(WINS) else r1
        for n in range(D // 128):
            ns = slice(128 * n, 128 * (n + 1))
            mf_v[n, lo:hi, :] = parts[j][lo - r0:hi - r0, ns]
            if j + 1 < len(WINS):
                n0 = WINS[j + 1][0]
                mf_v[n, hi:r1, :] = parts[j][hi - r0:r1 - r0, ns] + parts[j + 1][0:r1 - n0, ns]
    for n in range(D // 128):
        _permute_rows(m_v, mf_v.at[n], slice(128 * n, 128 * (n + 1)), bf16)

    pq0.append(qproj(xn_all[TM // 2:TM, :]))
    pqn0 = [_normalize(p, zrow) for p in pq0]
    resid_ln(0, 0, jnp.dot(pqn0[0], m_v[...], preferred_element_type=f32), 0)
    q4 = TM // 4
    for hh in range(2):
        resid_ln(0, 0, jnp.dot(pqn0[1][hh * q4:(hh + 1) * q4, :], m_v[...], preferred_element_type=f32),
                 TM // 2 + hh * q4)
    c_wg.wait()
    c_wu.wait()
    c_wd.wait()

    def gu(hn, c):
        g = jnp.dot(hn, wg_v[:, c * FC:(c + 1) * FC], preferred_element_type=f32)
        u = jnp.dot(hn, wu_v[:, c * FC:(c + 1) * FC], preferred_element_type=f32)
        return (jnp.maximum(g, 0.0) * u).astype(bf16)

    def down(a, c):
        return jnp.dot(a, wd_v[c * FC:(c + 1) * FC, :], preferred_element_type=f32)

    def phase2(i, carry):
        s = i % 2
        r = pl.multiple_of(i * TM, TM)
        rn = pl.multiple_of((i + 1) * TM, TM)
        hn = hn_buf[s]
        a0 = gu(hn, 0)
        pqn = _normalize(qproj(xn_all[pl.ds(rn, TM), :]), zrow_v[0:1, :])
        acc = down(a0, 0)
        a1 = gu(hn, 1)
        acc = acc + down(a1, 1)
        a2 = gu(hn, 2)
        attn = jnp.dot(pqn, m_v[...], preferred_element_type=f32)
        resid_ln(i + 1, 1 - s, attn)
        acc = acc + down(a2, 2)
        out_v[pl.ds(r, TM), :] = (acc + h_buf[s]).astype(bf16)
        o_copy(r, TM).start()
        return carry

    lax.fori_loop(0, NB - 1, phase2, 0)

    sl = (NB - 1) % 2
    hn = hn_buf[sl]
    acc = h_buf[sl]
    for c in range(F // FC - 1):
        acc = acc + down(gu(hn, c), c)
    a2 = gu(hn, F // FC - 1)
    r0 = (NB - 1) * TM
    for p0, p1 in TAIL:
        out_v[r0 + p0:r0 + p1, :] = (acc[p0:p1, :] + down(a2[p0:p1, :], F // FC - 1)).astype(bf16)
        o_copy(r0 + p0, p1 - p0).start()
    o_copy(0, S).wait()


@jax.jit
def pallas_sequential_preLN__linear_attn_block__glu_gated_reglu__prompt_kernel(
    A_x: jax.Array,
    A_wqkv: jax.Array,
    A_wo: jax.Array,
    B_x: jax.Array,
    B_W_gate: jax.Array,
    B_W_up: jax.Array,
    B_W_down: jax.Array,
):
    del B_x
    bf16, f32 = jnp.bfloat16, jnp.float32
    any_spec = pl.BlockSpec(memory_space=pl.ANY)
    return pl.pallas_call(
        _kernel,
        out_shape=jax.ShapeDtypeStruct((1, S, D), bf16),
        in_specs=[any_spec] * 6,
        out_specs=any_spec,
        scratch_shapes=[
            pltpu.VMEM((S, D), bf16),
            pltpu.VMEM((D, D), bf16),
            pltpu.VMEM((D, 2 * D), bf16),
            pltpu.VMEM((D, D), bf16),
            pltpu.VMEM((D, F), bf16),
            pltpu.VMEM((D, F), bf16),
            pltpu.VMEM((F, D), bf16),
            pltpu.VMEM((S, D), bf16),
            pltpu.VMEM((D, D), bf16),
            pltpu.VMEM((D, D), bf16),
            pltpu.VMEM((KC, D, 128), f32),
            pltpu.VMEM((S, D), bf16),
            pltpu.VMEM((2, TM, D), f32),
            pltpu.VMEM((2, TM, D), bf16),
            pltpu.VMEM((TM, D), bf16),
            pltpu.VMEM((TM, D), bf16),
            pltpu.VMEM((D, TM), bf16),
            pltpu.VMEM((D, TM), bf16),
            pltpu.VMEM((TM, D), bf16),
            pltpu.VMEM((TM, D), bf16),
            pltpu.VMEM((TM, D), f32),
            pltpu.VMEM((D, TM), f32),
            pltpu.VMEM((D, D), f32),
            pltpu.VMEM((D, 128), f32),
            pltpu.VMEM((D, 128), f32),
            pltpu.VMEM((8, D), f32),
            pltpu.VMEM((D // 128, D, 128), f32),
            pltpu.VMEM((D, D), bf16),
            pltpu.SemaphoreType.DMA((4,)),
            pltpu.SemaphoreType.DMA((2,)),
            pltpu.SemaphoreType.DMA((2,)),
            pltpu.SemaphoreType.DMA((1,)),
        ],
        compiler_params=pltpu.CompilerParams(vmem_limit_bytes=64 * 1024 * 1024),
    )(A_x, A_wqkv, A_wo, B_W_gate, B_W_up, B_W_down)
```

```python
import jax
import jax.numpy as jnp
from jax import lax
import jax.experimental.pallas as pl
import jax.experimental.pallas.tpu as pltpu

S, D, F = 2048, 640, 1536
H, DH = 32, 20
TM = 256
NB = S // TM
FC = 512
KC = D // 128
RC = 32
TAIL = ((0, 112), (112, 192), (192, 240), (240, 256))
LN_EPS = 1e-5
EPS = 1e-6
_NT = (((1,), (1,)), ((), ()))


def _row_windows():
    wins = []
    for j in range(D // 128):
        h0 = (128 * j) // DH
        h1 = (128 * j + 127) // DH
        r0 = (h0 * DH) // 16 * 16
        r1 = -(-((h1 + 1) * DH) // 16) * 16
        wins.append((r0, r1))
    return wins


WINS = _row_windows()


def _ln(x):
    m = jnp.mean(x, axis=-1, keepdims=True)
    xc = x - m
    v = jnp.mean(xc * xc, axis=-1, keepdims=True)
    return xc * lax.rsqrt(v + LN_EPS)


def _phi(t):
    return jnp.where(t > 0, t + 1.0, jnp.exp(t)) + EPS


def _head(i):
    return (i * 3277) >> 16


def _permute_rows(dst, src, cols, dtype):
    for m in range(DH):
        dst[32 * m:32 * (m + 1), cols] = src[pl.ds(m, H, stride=DH), :].astype(dtype)


def _normalize(pq, zrow):
    t = pq * zrow
    s = t[:, 0:128]
    for j in range(1, D // 128):
        s = s + t[:, 128 * j:128 * (j + 1)]
    s = s + pltpu.roll(s, 32, 1)
    s = s + pltpu.roll(s, 64, 1)
    rec = 1.0 / (s + EPS)
    parts = [(pq[:, 128 * j:128 * (j + 1)] * rec).astype(jnp.bfloat16) for j in range(D // 128)]
    return jnp.concatenate(parts, axis=1)


def _kernel(x_hbm, wqkv_hbm, wo_hbm, wg_hbm, wu_hbm, wd_hbm, out_hbm,
            x_v, wq_v, wk_v, wv_v, wo_v, wg_v, wu_v, wd_v, out_v,
            wkt_v, wqt_v, tq_v, xn_all, h_buf, hn_buf, xn_0, xn_1, pkt_v,
            kt_acc, g_v, gb_v, zacc_v, zp_v, zrow_v, mf_v, m_v,
            xsem, csem, wsem, osem):
    f32, bf16 = jnp.float32, jnp.bfloat16

    def x_copy(i):
        return pltpu.make_async_copy(x_hbm.at[0, pl.ds(i * TM, TM), :], x_v.at[pl.ds(i * TM, TM), :], xsem.at[0])

    def x2_copy(j):
        r = (2 * j + 2) * TM
        return pltpu.make_async_copy(x_hbm.at[0, pl.ds(r, 2 * TM), :], x_v.at[pl.ds(r, 2 * TM), :], xsem.at[1 + j])

    def o_copy(r, n):
        return pltpu.make_async_copy(out_v.at[pl.ds(r, n), :], out_hbm.at[0, pl.ds(r, n), :], osem.at[0])

    def c_copy(c):
        return pltpu.make_async_copy(wqkv_hbm.at[pl.ds(128 * c, 128), pl.ds(D, D)],
                                     wk_v.at[pl.ds(128 * c, 128), :], csem.at[c % 2])

    c_wq = pltpu.make_async_copy(wqkv_hbm.at[:, pl.ds(0, D)], wq_v, wsem.at[0])
    c_wv = pltpu.make_async_copy(wqkv_hbm.at[:, pl.ds(2 * D, D)], wv_v, wsem.at[0])
    c_wo = pltpu.make_async_copy(wo_hbm, wo_v, wsem.at[0])
    c_wg = pltpu.make_async_copy(wg_hbm, wg_v, wsem.at[1])
    c_wu = pltpu.make_async_copy(wu_hbm, wu_v, wsem.at[1])
    c_wd = pltpu.make_async_copy(wd_hbm, wd_v, wsem.at[1])

    x_copy(0).start()
    c_copy(0).start()

    g_v[...] = jnp.zeros_like(g_v)

    def prep1(i, dst, chains=0):
        toks = [None] * max(chains, 1)
        for k in range(TM // RC):
            r = pl.multiple_of(i * TM + k * RC, RC)
            x = x_v[pl.ds(r, RC), :].astype(f32)
            tok = toks[k % len(toks)]
            if tok is not None:
                x = jnp.concatenate([x[:, :D - 128], x[:, D - 128:] + tok], axis=1)
            xn = _ln(x)
            if chains:
                toks[k % len(toks)] = xn[:, D - 128:] * 0.0
            xn = xn.astype(bf16)
            dst[k * RC:(k + 1) * RC, :] = xn
            xn_all[pl.ds(r, RC), :] = xn

    def resid_ln(i, slot, attn, row0=0):
        for k in range(attn.shape[0] // RC):
            r = pl.multiple_of(i * TM + row0 + k * RC, RC)
            h = x_v[pl.ds(r, RC), :].astype(f32) + attn[k * RC:(k + 1) * RC, :]
            h_buf[slot, row0 + k * RC:row0 + (k + 1) * RC, :] = h
            hn_buf[slot, row0 + k * RC:row0 + (k + 1) * RC, :] = _ln(h).astype(bf16)

    def gacc(pkt, xn):
        hs = [slice(hh * (D // 2), (hh + 1) * (D // 2)) for hh in range(2)]
        gs = [jnp.dot(pkt[rs, 0:128], xn[0:128, :], preferred_element_type=f32) for rs in hs]
        for c in range(1, TM // 128):
            gs = [g + jnp.dot(pkt[rs, 128 * c:128 * (c + 1)], xn[128 * c:128 * (c + 1), :],
                              preferred_element_type=f32) for g, rs in zip(gs, hs)]
        for g, rs in zip(gs, hs):
            g_v[rs, :] += g

    def zfold(pkt):
        zs = pkt[:, 0:128]
        for c in range(1, TM // 128):
            zs = zs + pkt[:, 128 * c:128 * (c + 1)]
        return zs

    def kpart(c):
        kp = slice(128 * c, 128 * (c + 1))
        xc = xn_0[:, kp]
        for hh in range(2):
            rs = slice(hh * (D // 2), (hh + 1) * (D // 2))
            ktp = lax.dot_general(wkt_v[rs, kp], xc, _NT, preferred_element_type=f32)
            if c == 0:
                kt_acc[rs, :] = ktp
            else:
                kt_acc[rs, :] += ktp

    def kproj(xn_c, pkt_dst):
        for c in range(TM // 128):
            cs = slice(128 * c, 128 * (c + 1))
            xn = xn_c[cs, :]
            for hh in range(2):
                rs = slice(hh * (D // 2), (hh + 1) * (D // 2))
                pkt = _phi(lax.dot_general(wkt_v[rs, :], xn, _NT, preferred_element_type=f32))
                zacc_v[rs, :] += pkt
                pkt_dst[rs, cs] = pkt.astype(bf16)

    def qproj(xn):
        return _phi(lax.dot_general(xn, wqt_v[...], _NT, preferred_element_type=f32))

    x_copy(0).wait()
    c_copy(1).start()
    prep1(0, xn_0)
    for c in range(KC):
        c_copy(c).wait()
        if c + 2 < KC:
            c_copy(c + 2).start()
        elif c + 2 == KC:
            x_copy(1).start()
        else:
            x2_copy(0).start()
        ks = slice(128 * c, 128 * (c + 1))
        if c > 0:
            kpart(c - 1)
        wkt_v[:, ks] = wk_v[ks, :].astype(f32).T.astype(bf16)
    kpart(KC - 1)
    pkt0 = _phi(kt_acc[...])
    zacc_v[...] = zfold(pkt0)
    pkt_v[...] = pkt0.astype(bf16)
    x_copy(1).wait()
    x2_copy(1).start()
    x2_copy(2).start()
    prep1(1, xn_1, chains=2)
    gacc(pkt_v, xn_0)

    c_wq.start()
    c_wv.start()
    c_wo.start()
    c_wg.start()
    c_wu.start()
    c_wd.start()

    def phase1(j, carry):
        x2_copy(j).wait()
        prep1(2 * j + 2, xn_0, chains=1)
        kproj(xn_1, pkt_v)
        gacc(pkt_v, xn_1)
        prep1(2 * j + 3, xn_1, chains=1)
        kproj(xn_0, pkt_v)
        gacc(pkt_v, xn_0)
        return carry

    lax.fori_loop(0, NB // 2 - 1, phase1, 0)

    c_wq.wait()
    c_wv.wait()
    c_wo.wait()
    for c in range(KC):
        ks = slice(128 * c, 128 * (c + 1))
        tq_v[c] = wq_v[ks, :].astype(f32).T
        _permute_rows(wqt_v, tq_v.at[c], ks, bf16)
    kproj(xn_1, pkt_v)
    q4 = TM // 4
    pq0 = [qproj(xn_all[0:q4, :])]
    gacc(pkt_v, xn_1)
    gb_v[...] = g_v[...].astype(bf16)
    pq0.append(qproj(xn_all[q4:2 * q4, :]))

    _permute_rows(zp_v, zacc_v, slice(None), f32)
    zrow = jnp.sum(zp_v[...].T, axis=0, keepdims=True)
    zrow_v[...] = jnp.broadcast_to(zrow, zrow_v.shape)
    kvms = []
    for j, (r0, r1) in enumerate(WINS):
        rows = lax.broadcasted_iota(jnp.int32, (r1 - r0, 128), 0) + r0
        cols = lax.broadcasted_iota(jnp.int32, (r1 - r0, 128), 1) + 128 * j
        kv = jnp.dot(gb_v[r0:r1, :], wv_v[:, 128 * j:128 * (j + 1)], preferred_element_type=f32)
        kvms.append(jnp.where(_head(rows) == _head(cols), kv, 0.0).astype(bf16))
    pq0.append(qproj(xn_all[2 * q4:3 * q4, :]))
    parts = [jnp.dot(kvms[j], wo_v[128 * j:128 * (j + 1), :], preferred_element_type=f32)
             for j in range(len(WINS))]
    for j, (r0, r1) in enumerate(WINS):
        lo = WINS[j - 1][1] if j > 0 else r0
        hi = WINS[j + 1][0] if j + 1 < len(WINS) else r1
        for n in range(D // 128):
            ns = slice(128 * n, 128 * (n + 1))
            mf_v[n, lo:hi, :] = parts[j][lo - r0:hi - r0, ns]
            if j + 1 < len(WINS):
                n0 = WINS[j + 1][0]
                mf_v[n, hi:r1, :] = parts[j][hi - r0:r1 - r0, ns] + parts[j + 1][0:r1 - n0, ns]
    for n in range(D // 128):
        _permute_rows(m_v, mf_v.at[n], slice(128 * n, 128 * (n + 1)), bf16)
    pq0.append(qproj(xn_all[3 * q4:TM, :]))
    pqn0 = [_normalize(p, zrow) for p in pq0]
    resid_ln(0, 0, jnp.dot(jnp.concatenate(pqn0[0:2], axis=0), m_v[...], preferred_element_type=f32), 0)
    for hh in range(2, 4):
        resid_ln(0, 0, jnp.dot(pqn0[hh], m_v[...], preferred_element_type=f32), hh * q4)
    c_wg.wait()
    c_wu.wait()
    c_wd.wait()

    def gu(hn, c):
        g = jnp.dot(hn, wg_v[:, c * FC:(c + 1) * FC], preferred_element_type=f32)
        u = jnp.dot(hn, wu_v[:, c * FC:(c + 1) * FC], preferred_element_type=f32)
        return (jnp.maximum(g, 0.0) * u).astype(bf16)

    def down(a, c):
        return jnp.dot(a, wd_v[c * FC:(c + 1) * FC, :], preferred_element_type=f32)

    def phase2(i, carry):
        s = i % 2
        r = pl.multiple_of(i * TM, TM)
        rn = pl.multiple_of((i + 1) * TM, TM)
        hn = hn_buf[s]
        a0 = gu(hn, 0)
        pqn = _normalize(qproj(xn_all[pl.ds(rn, TM), :]), zrow_v[0:1, :])
        acc = down(a0, 0)
        a1 = gu(hn, 1)
        acc = acc + down(a1, 1)
        a2 = gu(hn, 2)
        attn = jnp.dot(pqn, m_v[...], preferred_element_type=f32)
        resid_ln(i + 1, 1 - s, attn)
        acc = acc + down(a2, 2)
        out_v[pl.ds(r, TM), :] = (acc + h_buf[s]).astype(bf16)
        o_copy(r, TM).start()
        return carry

    lax.fori_loop(0, NB - 1, phase2, 0)

    sl = (NB - 1) % 2
    hn = hn_buf[sl]
    acc = h_buf[sl]
    for c in range(F // FC - 1):
        acc = acc + down(gu(hn, c), c)
    a2 = gu(hn, F // FC - 1)
    r0 = (NB - 1) * TM
    for p0, p1 in TAIL:
        out_v[r0 + p0:r0 + p1, :] = (acc[p0:p1, :] + down(a2[p0:p1, :], F // FC - 1)).astype(bf16)
        o_copy(r0 + p0, p1 - p0).start()
    o_copy(0, S).wait()


@jax.jit
def pallas_sequential_preLN__linear_attn_block__glu_gated_reglu__prompt_kernel(
    A_x: jax.Array,
    A_wqkv: jax.Array,
    A_wo: jax.Array,
    B_x: jax.Array,
    B_W_gate: jax.Array,
    B_W_up: jax.Array,
    B_W_down: jax.Array,
):
    del B_x
    bf16, f32 = jnp.bfloat16, jnp.float32
    any_spec = pl.BlockSpec(memory_space=pl.ANY)
    return pl.pallas_call(
        _kernel,
        out_shape=jax.ShapeDtypeStruct((1, S, D), bf16),
        in_specs=[any_spec] * 6,
        out_specs=any_spec,
        scratch_shapes=[
            pltpu.VMEM((S, D), bf16),
            pltpu.VMEM((D, D), bf16),
            pltpu.VMEM((D, D), bf16),
            pltpu.VMEM((D, D), bf16),
            pltpu.VMEM((D, D), bf16),
            pltpu.VMEM((D, F), bf16),
            pltpu.VMEM((D, F), bf16),
            pltpu.VMEM((F, D), bf16),
            pltpu.VMEM((S, D), bf16),
            pltpu.VMEM((D, D), bf16),
            pltpu.VMEM((D, D), bf16),
            pltpu.VMEM((KC, D, 128), f32),
            pltpu.VMEM((S, D), bf16),
            pltpu.VMEM((2, TM, D), f32),
            pltpu.VMEM((2, TM, D), bf16),
            pltpu.VMEM((TM, D), bf16),
            pltpu.VMEM((TM, D), bf16),
            pltpu.VMEM((D, TM), bf16),
            pltpu.VMEM((D, TM), f32),
            pltpu.VMEM((D, D), f32),
            pltpu.VMEM((D, D), bf16),
            pltpu.VMEM((D, 128), f32),
            pltpu.VMEM((D, 128), f32),
            pltpu.VMEM((8, D), f32),
            pltpu.VMEM((D // 128, D, 128), f32),
            pltpu.VMEM((D, D), bf16),
            pltpu.SemaphoreType.DMA((4,)),
            pltpu.SemaphoreType.DMA((2,)),
            pltpu.SemaphoreType.DMA((2,)),
            pltpu.SemaphoreType.DMA((1,)),
        ],
        compiler_params=pltpu.CompilerParams(vmem_limit_bytes=64 * 1024 * 1024),
    )(A_x, A_wqkv, A_wo, B_W_gate, B_W_up, B_W_down)
```

```python
import jax
import jax.numpy as jnp
from jax import lax
import jax.experimental.pallas as pl
import jax.experimental.pallas.tpu as pltpu

S, D, F = 2048, 640, 1536
H, DH = 32, 20
TM = 256
NB = S // TM
FC = 512
KC = D // 128
RC = 32
TAIL = ((0, 112), (112, 192), (192, 240), (240, 256))
LN_EPS = 1e-5
EPS = 1e-6
_NT = (((1,), (1,)), ((), ()))


def _row_windows():
    wins = []
    for j in range(D // 128):
        h0 = (128 * j) // DH
        h1 = (128 * j + 127) // DH
        r0 = (h0 * DH) // 16 * 16
        r1 = -(-((h1 + 1) * DH) // 16) * 16
        wins.append((r0, r1))
    return wins


WINS = _row_windows()


def _ln(x):
    m = jnp.mean(x, axis=-1, keepdims=True)
    xc = x - m
    v = jnp.mean(xc * xc, axis=-1, keepdims=True)
    return xc * lax.rsqrt(v + LN_EPS)


def _phi(t):
    return jnp.where(t > 0, t + 1.0, jnp.exp(t)) + EPS


def _head(i):
    return (i * 3277) >> 16


def _permute_rows(dst, src, cols, dtype):
    for m in range(DH):
        dst[32 * m:32 * (m + 1), cols] = src[pl.ds(m, H, stride=DH), :].astype(dtype)


def _normalize(pq, zrow):
    t = pq * zrow
    s = t[:, 0:128]
    for j in range(1, D // 128):
        s = s + t[:, 128 * j:128 * (j + 1)]
    s = s + pltpu.roll(s, 32, 1)
    s = s + pltpu.roll(s, 64, 1)
    rec = 1.0 / (s + EPS)
    parts = [(pq[:, 128 * j:128 * (j + 1)] * rec).astype(jnp.bfloat16) for j in range(D // 128)]
    return jnp.concatenate(parts, axis=1)


def _kernel(x_hbm, wqkv_hbm, wo_hbm, wg_hbm, wu_hbm, wd_hbm, out_hbm,
            x_v, wq_v, wk_v, wv_v, wo_v, wg_v, wu_v, wd_v, out_v,
            wkt_v, wqt_v, tq_v, xn_all, h_buf, hn_buf, xn_0, xn_1, pkt_v,
            kt_acc, g_v, gb_v, zacc_v, zp_v, zrow_v, mf_v, m_v,
            xsem, csem, wsem, osem):
    f32, bf16 = jnp.float32, jnp.bfloat16

    def x_copy(i):
        return pltpu.make_async_copy(x_hbm.at[0, pl.ds(i * TM, TM), :], x_v.at[pl.ds(i * TM, TM), :], xsem.at[0])

    def x2_copy(j):
        r = (2 * j + 2) * TM
        return pltpu.make_async_copy(x_hbm.at[0, pl.ds(r, 2 * TM), :], x_v.at[pl.ds(r, 2 * TM), :], xsem.at[1 + j])

    def o_copy(r, n):
        return pltpu.make_async_copy(out_v.at[pl.ds(r, n), :], out_hbm.at[0, pl.ds(r, n), :], osem.at[0])

    def c_copy(c):
        return pltpu.make_async_copy(wqkv_hbm.at[pl.ds(128 * c, 128), pl.ds(D, D)],
                                     wk_v.at[pl.ds(128 * c, 128), :], csem.at[c % 2])

    c_wq = pltpu.make_async_copy(wqkv_hbm.at[:, pl.ds(0, D)], wq_v, wsem.at[0])
    c_wv = pltpu.make_async_copy(wqkv_hbm.at[:, pl.ds(2 * D, D)], wv_v, wsem.at[0])
    c_wo = pltpu.make_async_copy(wo_hbm, wo_v, wsem.at[0])
    c_wg = pltpu.make_async_copy(wg_hbm, wg_v, wsem.at[1])
    c_wu = pltpu.make_async_copy(wu_hbm, wu_v, wsem.at[1])
    c_wd = pltpu.make_async_copy(wd_hbm, wd_v, wsem.at[1])

    x_copy(0).start()
    c_copy(0).start()

    g_v[...] = jnp.zeros_like(g_v)

    def prep1(i, dst, chains=0):
        toks = [None] * max(chains, 1)
        for k in range(TM // RC):
            r = pl.multiple_of(i * TM + k * RC, RC)
            x = x_v[pl.ds(r, RC), :].astype(f32)
            tok = toks[k % len(toks)]
            if tok is not None:
                x = jnp.concatenate([x[:, :D - 128], x[:, D - 128:] + tok], axis=1)
            xn = _ln(x)
            if chains:
                toks[k % len(toks)] = xn[:, D - 128:] * 0.0
            xn = xn.astype(bf16)
            dst[k * RC:(k + 1) * RC, :] = xn
            xn_all[pl.ds(r, RC), :] = xn

    def resid_ln(i, slot, attn, row0=0):
        for k in range(attn.shape[0] // RC):
            r = pl.multiple_of(i * TM + row0 + k * RC, RC)
            h = x_v[pl.ds(r, RC), :].astype(f32) + attn[k * RC:(k + 1) * RC, :]
            h_buf[slot, row0 + k * RC:row0 + (k + 1) * RC, :] = h
            hn_buf[slot, row0 + k * RC:row0 + (k + 1) * RC, :] = _ln(h).astype(bf16)

    def gacc(pkt, xn, last=False):
        hs = [slice(hh * (D // 2), (hh + 1) * (D // 2)) for hh in range(2)]
        gs = [jnp.dot(pkt[rs, 0:128], xn[0:128, :], preferred_element_type=f32) for rs in hs]
        for c in range(1, TM // 128):
            gs = [g + jnp.dot(pkt[rs, 128 * c:128 * (c + 1)], xn[128 * c:128 * (c + 1), :],
                              preferred_element_type=f32) for g, rs in zip(gs, hs)]
        for g, rs in zip(gs, hs):
            if last:
                gb_v[rs, :] = (g_v[rs, :] + g).astype(bf16)
            else:
                g_v[rs, :] += g

    def zfold(pkt):
        zs = pkt[:, 0:128]
        for c in range(1, TM // 128):
            zs = zs + pkt[:, 128 * c:128 * (c + 1)]
        return zs

    def kpart(c):
        kp = slice(128 * c, 128 * (c + 1))
        xc = xn_0[:, kp]
        for hh in range(2):
            rs = slice(hh * (D // 2), (hh + 1) * (D // 2))
            ktp = lax.dot_general(wkt_v[rs, kp], xc, _NT, preferred_element_type=f32)
            if c == 0:
                kt_acc[rs, :] = ktp
            else:
                kt_acc[rs, :] += ktp

    def kproj(xn_c, pkt_dst):
        for c in range(TM // 128):
            cs = slice(128 * c, 128 * (c + 1))
            xn = xn_c[cs, :]
            for hh in range(2):
                rs = slice(hh * (D // 2), (hh + 1) * (D // 2))
                pkt = _phi(lax.dot_general(wkt_v[rs, :], xn, _NT, preferred_element_type=f32))
                zacc_v[rs, :] += pkt
                pkt_dst[rs, cs] = pkt.astype(bf16)

    def qproj(xn):
        return _phi(lax.dot_general(xn, wqt_v[...], _NT, preferred_element_type=f32))

    x_copy(0).wait()
    c_copy(1).start()
    prep1(0, xn_0)
    for c in range(KC):
        c_copy(c).wait()
        if c + 2 < KC:
            c_copy(c + 2).start()
        elif c + 2 == KC:
            x_copy(1).start()
        else:
            x2_copy(0).start()
        ks = slice(128 * c, 128 * (c + 1))
        if c > 0:
            kpart(c - 1)
        wkt_v[:, ks] = wk_v[ks, :].astype(f32).T.astype(bf16)
    kpart(KC - 1)
    pkt0 = _phi(kt_acc[...])
    zacc_v[...] = zfold(pkt0)
    pkt_v[...] = pkt0.astype(bf16)
    x_copy(1).wait()
    x2_copy(1).start()
    x2_copy(2).start()
    prep1(1, xn_1, chains=2)
    gacc(pkt_v, xn_0)

    c_wq.start()
    c_wv.start()
    c_wo.start()
    c_wg.start()
    c_wu.start()
    c_wd.start()

    def phase1(j, carry):
        x2_copy(j).wait()
        prep1(2 * j + 2, xn_0, chains=1)
        kproj(xn_1, pkt_v)
        gacc(pkt_v, xn_1)
        prep1(2 * j + 3, xn_1, chains=1)
        kproj(xn_0, pkt_v)
        gacc(pkt_v, xn_0)
        return carry

    lax.fori_loop(0, NB // 2 - 1, phase1, 0)

    c_wq.wait()
    c_wv.wait()
    c_wo.wait()
    for c in range(KC):
        ks = slice(128 * c, 128 * (c + 1))
        tq_v[c] = wq_v[ks, :].astype(f32).T
        _permute_rows(wqt_v, tq_v.at[c], ks, bf16)
    kproj(xn_1, pkt_v)
    q4 = TM // 4
    pq0 = [qproj(xn_all[0:q4, :])]
    gacc(pkt_v, xn_1, last=True)
    pq0.append(qproj(xn_all[q4:2 * q4, :]))

    _permute_rows(zp_v, zacc_v, slice(None), f32)
    zrow = jnp.sum(zp_v[...].T, axis=0, keepdims=True)
    zrow_v[...] = jnp.broadcast_to(zrow, zrow_v.shape)
    kvms = []
    for j, (r0, r1) in enumerate(WINS):
        rows = lax.broadcasted_iota(jnp.int32, (r1 - r0, 128), 0) + r0
        cols = lax.broadcasted_iota(jnp.int32, (r1 - r0, 128), 1) + 128 * j
        kv = jnp.dot(gb_v[r0:r1, :], wv_v[:, 128 * j:128 * (j + 1)], preferred_element_type=f32)
        kvms.append(jnp.where(_head(rows) == _head(cols), kv, 0.0).astype(bf16))
    pq0.append(qproj(xn_all[2 * q4:3 * q4, :]))
    parts = [jnp.dot(kvms[j], wo_v[128 * j:128 * (j + 1), :], preferred_element_type=f32)
             for j in range(len(WINS))]
    for j, (r0, r1) in enumerate(WINS):
        lo = WINS[j - 1][1] if j > 0 else r0
        hi = WINS[j + 1][0] if j + 1 < len(WINS) else r1
        for n in range(D // 128):
            ns = slice(128 * n, 128 * (n + 1))
            mf_v[n, lo:hi, :] = parts[j][lo - r0:hi - r0, ns]
            if j + 1 < len(WINS):
                n0 = WINS[j + 1][0]
                mf_v[n, hi:r1, :] = parts[j][hi - r0:r1 - r0, ns] + parts[j + 1][0:r1 - n0, ns]
    for n in range(D // 128):
        _permute_rows(m_v, mf_v.at[n], slice(128 * n, 128 * (n + 1)), bf16)
    pq0.append(qproj(xn_all[3 * q4:TM, :]))
    pqn0 = [_normalize(p, zrow) for p in pq0]
    resid_ln(0, 0, jnp.dot(jnp.concatenate(pqn0[0:2], axis=0), m_v[...], preferred_element_type=f32), 0)
    for hh in range(2, 4):
        resid_ln(0, 0, jnp.dot(pqn0[hh], m_v[...], preferred_element_type=f32), hh * q4)
    c_wg.wait()
    c_wu.wait()
    c_wd.wait()

    def gu(hn, c):
        g = jnp.dot(hn, wg_v[:, c * FC:(c + 1) * FC], preferred_element_type=f32)
        u = jnp.dot(hn, wu_v[:, c * FC:(c + 1) * FC], preferred_element_type=f32)
        return (jnp.maximum(g, 0.0) * u).astype(bf16)

    def down(a, c):
        return jnp.dot(a, wd_v[c * FC:(c + 1) * FC, :], preferred_element_type=f32)

    def phase2(i, carry):
        s = i % 2
        r = pl.multiple_of(i * TM, TM)
        rn = pl.multiple_of((i + 1) * TM, TM)
        hn = hn_buf[s]
        a0 = gu(hn, 0)
        pqn = _normalize(qproj(xn_all[pl.ds(rn, TM), :]), zrow_v[0:1, :])
        acc = down(a0, 0)
        a1 = gu(hn, 1)
        acc = acc + down(a1, 1)
        a2 = gu(hn, 2)
        attn = jnp.dot(pqn, m_v[...], preferred_element_type=f32)
        resid_ln(i + 1, 1 - s, attn)
        acc = acc + down(a2, 2)
        out_v[pl.ds(r, TM), :] = (acc + h_buf[s]).astype(bf16)
        o_copy(r, TM).start()
        return carry

    lax.fori_loop(0, NB - 1, phase2, 0)

    sl = (NB - 1) % 2
    hn = hn_buf[sl]
    acc = h_buf[sl]
    for c in range(F // FC - 1):
        acc = acc + down(gu(hn, c), c)
    a2 = gu(hn, F // FC - 1)
    r0 = (NB - 1) * TM
    for p0, p1 in TAIL:
        out_v[r0 + p0:r0 + p1, :] = (acc[p0:p1, :] + down(a2[p0:p1, :], F // FC - 1)).astype(bf16)
        o_copy(r0 + p0, p1 - p0).start()
    o_copy(0, S).wait()


@jax.jit
def pallas_sequential_preLN__linear_attn_block__glu_gated_reglu__prompt_kernel(
    A_x: jax.Array,
    A_wqkv: jax.Array,
    A_wo: jax.Array,
    B_x: jax.Array,
    B_W_gate: jax.Array,
    B_W_up: jax.Array,
    B_W_down: jax.Array,
):
    del B_x
    bf16, f32 = jnp.bfloat16, jnp.float32
    any_spec = pl.BlockSpec(memory_space=pl.ANY)
    return pl.pallas_call(
        _kernel,
        out_shape=jax.ShapeDtypeStruct((1, S, D), bf16),
        in_specs=[any_spec] * 6,
        out_specs=any_spec,
        scratch_shapes=[
            pltpu.VMEM((S, D), bf16),
            pltpu.VMEM((D, D), bf16),
            pltpu.VMEM((D, D), bf16),
            pltpu.VMEM((D, D), bf16),
            pltpu.VMEM((D, D), bf16),
            pltpu.VMEM((D, F), bf16),
            pltpu.VMEM((D, F), bf16),
            pltpu.VMEM((F, D), bf16),
            pltpu.VMEM((S, D), bf16),
            pltpu.VMEM((D, D), bf16),
            pltpu.VMEM((D, D), bf16),
            pltpu.VMEM((KC, D, 128), f32),
            pltpu.VMEM((S, D), bf16),
            pltpu.VMEM((2, TM, D), f32),
            pltpu.VMEM((2, TM, D), bf16),
            pltpu.VMEM((TM, D), bf16),
            pltpu.VMEM((TM, D), bf16),
            pltpu.VMEM((D, TM), bf16),
            pltpu.VMEM((D, TM), f32),
            pltpu.VMEM((D, D), f32),
            pltpu.VMEM((D, D), bf16),
            pltpu.VMEM((D, 128), f32),
            pltpu.VMEM((D, 128), f32),
            pltpu.VMEM((8, D), f32),
            pltpu.VMEM((D // 128, D, 128), f32),
            pltpu.VMEM((D, D), bf16),
            pltpu.SemaphoreType.DMA((4,)),
            pltpu.SemaphoreType.DMA((2,)),
            pltpu.SemaphoreType.DMA((2,)),
            pltpu.SemaphoreType.DMA((1,)),
        ],
        compiler_params=pltpu.CompilerParams(vmem_limit_bytes=64 * 1024 * 1024),
    )(A_x, A_wqkv, A_wo, B_W_gate, B_W_up, B_W_down)
```
